```python
import os as _os
_os.environ.setdefault("JAX_PLATFORMS", "cpu")
import jax
import jax.numpy as jnp

def _softmax(x, axis=-1):
    return jax.nn.softmax(x, axis=axis)
def _gelu(x):
    return jax.nn.gelu(x, approximate=True)
def _silu(x):
    return jax.nn.silu(x)
def _sigmoid(x):
    return jax.nn.sigmoid(x)
def _layernorm(x, axis=-1, eps=1e-5):
    m = jnp.mean(x, axis=axis, keepdims=True)
    v = jnp.var(x, axis=axis, keepdims=True)
    return (x - m) / jnp.sqrt(v + eps)
def _scatter_add(tgt, idx, src, axis=0):
    return tgt.at[idx].add(src)
def _segment_sum(src, seg, n):
    return jax.ops.segment_sum(src, seg, n)
class _Rng:
    def __init__(self, key):
        self._k = key
    def _next(self):
        self._k, sub = jax.random.split(self._k)
        return sub
    def normal(self, shape):
        return jax.random.normal(self._next(), shape, dtype=jnp.bfloat16)
    def randint(self, lo, hi, shape):
        return jax.random.randint(self._next(), shape, lo, hi, dtype=jnp.int32)
    def uniform(self, shape, lo=0.0, hi=1.0):
        return jax.random.uniform(self._next(), shape, jnp.bfloat16, lo, hi)
    def permutation(self, n):
        return jax.random.permutation(self._next(), n)


kernel_name = 'parallel_sum__mha_block_cached__dense_activation_mish__decode'

def setup_inputs():
    _rng = _Rng(jax.random.key(int.from_bytes(__import__("os").urandom(4), "little")))
    _w = (lambda a: (lambda t: t.astype(jnp.bfloat16) if jnp.issubdtype(t.dtype, jnp.floating) else t)(jnp.asarray(a)))
    def _A_setup():
        B, Sq, D = 1, 1, 448
        H, Sk, Dh = 16, 16384, 256
        return {
            "x": _w((lambda *s: _rng.normal(s) * 0.05)(B, Sq, D)),
            "k_cache": _w((lambda *s: _rng.normal(s) * 1.6)(B, H, Sk, Dh)),
            "v_cache": _w((lambda *s: _rng.normal(s) * 0.8)(B, H, Sk, Dh)),
            "wq": _w((lambda *s: _rng.normal(s) * 1.6)(D, H * Dh) * (D ** -0.5)),
            "wo": _w((lambda *s: _rng.normal(s) * 0.8)(H * Dh, D) * ((H * Dh) ** -0.5)),
        }
    _A_in = _A_setup()

    def _B_setup():
        B, S, D, F = 1, 1, 448, 1792
        return {
            "x": _w((lambda *s: _rng.normal(s) * 0.05)(B, S, D)),
            "w1": _w((lambda *s: _rng.normal(s) * 0.8)(D, F) * (D ** -0.5)),
            "b1": _w((lambda *s: _rng.normal(s) * 0.05)(F)),
            "w2": _w((lambda *s: _rng.normal(s) * 0.05)(F, D) * (F ** -0.5)),
        }
    _B_in = _B_setup()

    return {
        "A_x": _A_in["x"],
        "A_k_cache": _A_in["k_cache"],
        "A_v_cache": _A_in["v_cache"],
        "A_wq": _A_in["wq"],
        "A_wo": _A_in["wo"],
        "B_x": _B_in["x"],
        "B_w1": _B_in["w1"],
        "B_b1": _B_in["b1"],
        "B_w2": _B_in["w2"],
    }

def reference(A_x, A_k_cache, A_v_cache, A_wq, A_wo, B_x, B_w1, B_b1, B_w2):
    def _A_ref(x, k_cache, v_cache, wq, wo):
        B, Sq, D = x.shape
        H, Dh = 16, 256
        q = (lambda x, *d: x.transpose(*d))((x @ wq).reshape(B, Sq, H, Dh), 0, 2, 1, 3)
        scores = jnp.einsum("bhqd,bhkd->bhqk", q, k_cache) * (Dh ** -0.5)
        p = _softmax(scores, axis=-1)
        o = jnp.einsum("bhqk,bhkd->bhqd", p, v_cache)
        return (lambda x, *d: x.transpose(*d))(o, 0, 2, 1, 3).reshape(B, Sq, H * Dh) @ wo

    def _B_ref(x, w1, b1, w2):
        h = jnp.einsum("bsd,df->bsf", x, w1) + b1
        sp = jnp.log1p(jnp.exp(-jnp.abs(h))) + jnp.where(h > 0, h, jnp.zeros_like(h))
        act = h * jnp.tanh(sp)
        return jnp.einsum("bsf,fd->bsd", act, w2)

    x = A_x
    xn = _layernorm(x, axis=-1)
    return x + _A_ref(xn, A_k_cache, A_v_cache, A_wq, A_wo) + _B_ref(xn, B_w1, B_b1, B_w2)
```

```python
import functools
import jax
import jax.numpy as jnp
from jax import lax
from jax.experimental import pallas as pl
from jax.experimental.pallas import tpu as pltpu

H, SK, DH, D, F = 16, 16384, 256, 448, 1792
NT = (((1,), (1,)), ((), ()))
f32, bf16 = jnp.float32, jnp.bfloat16


def build(S=8, RW=32, A=2, NP=8, U=1, name="k1", interpret=False):
    L = SK // S
    E = L // RW
    C = S * RW
    RING = 2 * NP

    def kern(x_hbm, k_hbm, v_hbm, wq_hbm, wot_hbm, w1_hbm, b1_hbm, w2t_hbm, o_ref,
             kbuf, vbuf, sbuf, qbuf, xbuf, wqbuf, wobuf, w1buf, b1buf, w2buf, ksem, vsem, wsem):
        def start(src, buf, sem, t):
            h = t // E
            r = pl.multiple_of((t % E) * RW, RW)
            slot = t % RING
            si = t % NP
            pltpu.make_async_copy(src.at[pl.ds(h * S, A), pl.ds(r, RW)], buf.at[slot, pl.ds(0, A)], sem.at[si]).start(priority=0)
            pltpu.make_async_copy(src.at[pl.ds(h * S + A, S - A), pl.ds(r, RW)], buf.at[slot, pl.ds(A, S - A)], sem.at[si]).start(priority=1)

        def wait(buf, sem, t):
            slot = t % RING
            pltpu.make_async_copy(buf.at[slot], buf.at[slot], sem.at[t % NP]).wait()

        wcopies = [pltpu.make_async_copy(s, d, wsem.at[i]) for i, (s, d) in enumerate(
            [(x_hbm, xbuf), (wq_hbm, wqbuf), (w1_hbm, w1buf), (b1_hbm, b1buf), (w2t_hbm, w2buf), (wot_hbm, wobuf)])]
        for c in wcopies:
            c.start(priority=1)
        for t in range(NP):
            start(k_hbm, kbuf, ksem, t)

        wcopies[0].wait()
        x = xbuf[0].astype(f32)
        mu = jnp.mean(x, axis=-1, keepdims=True)
        xc = x - mu
        var = jnp.mean(xc * xc, axis=-1, keepdims=True)
        xn = jnp.broadcast_to(xc / jnp.sqrt(var + 1e-5), (8, D)).astype(bf16)
        wcopies[1].wait()
        for h in range(H):
            q = jnp.dot(xn, wqbuf[:, h * DH:(h + 1) * DH], preferred_element_type=f32)
            qbuf[h] = q.astype(bf16).astype(f32) * (DH ** -0.5)
        wcopies[2].wait(); wcopies[3].wait()
        hid = jnp.dot(xn, w1buf[...], preferred_element_type=f32) + b1buf[...].astype(f32).reshape(1, F)
        sp = jnp.log1p(jnp.exp(-jnp.abs(hid))) + jnp.maximum(hid, 0.0)
        act = (hid * jnp.tanh(sp)).astype(bf16)
        wcopies[4].wait()
        out0 = x + lax.dot_general(act, w2buf[...], NT, preferred_element_type=f32)

        def k_step(h, j, q, mx):
            t = h * E + j
            wait(kbuf, ksem, t)
            return t

        def k_comp(t, j, h, q, mx):
            kb = kbuf[t % RING].reshape(C, DH)
            s = lax.dot_general(q, kb, NT, preferred_element_type=f32)
            sbuf[h % 2, j] = s
            for c in range(C // 128):
                mx = jnp.maximum(mx, s[:, c * 128:(c + 1) * 128])
            return mx

        def v_comp(t, j, h, m, l, acc):
            p = jnp.exp(sbuf[h % 2, j] - m)
            for c in range(C // 128):
                l = l + p[:, c * 128:(c + 1) * 128]
            vb = vbuf[t % RING].reshape(C, DH)
            acc = acc + jnp.dot(p.astype(bf16), vb, preferred_element_type=f32)
            return l, acc

        neg = jnp.full((8, 128), -jnp.inf, f32)
        zl = jnp.zeros((8, 128), f32)
        za = jnp.zeros((8, DH), f32)

        q0 = qbuf[0].astype(bf16)
        def first(j, mx):
            wait(kbuf, ksem, j)
            start(k_hbm, kbuf, ksem, j + NP)
            @pl.when(j >= E - NP)
            def _():
                start(v_hbm, vbuf, vsem, j - (E - NP))
            return k_comp(j, j, 0, q0, mx)
        mx = lax.fori_loop(0, E, first, neg)
        wcopies[5].wait()

        def finish(h, l, acc, out):
            o = (acc / jnp.sum(l, axis=-1, keepdims=True)).astype(bf16)
            w = wobuf[:, pl.ds(pl.multiple_of(h * DH, DH), DH)]
            return out + lax.dot_general(o, w, NT, preferred_element_type=f32)

        def head(h, carry):
            mx, out = carry
            m = jnp.max(mx, axis=-1, keepdims=True)
            q = qbuf[h + 1].astype(bf16)
            def body(jj, c):
                mx, l, acc = c
                for u in range(U):
                    j = jj * U + u
                    tk = (h + 1) * E + j
                    tv = h * E + j
                    wait(kbuf, ksem, tk)
                    @pl.when(tk + NP < H * E)
                    def _():
                        start(k_hbm, kbuf, ksem, tk + NP)
                    mx = k_comp(tk, j, h + 1, q, mx)
                    wait(vbuf, vsem, tv)
                    start(v_hbm, vbuf, vsem, tv + NP)
                    l, acc = v_comp(tv, j, h, m, l, acc)
                return mx, l, acc
            mx, l, acc = lax.fori_loop(0, E // U, body, (neg, zl, za))
            return mx, finish(h, l, acc, out)
        mx, out = lax.fori_loop(0, H - 1, head, (mx, out0))

        m = jnp.max(mx, axis=-1, keepdims=True)
        def last(j, c):
            tv = (H - 1) * E + j
            wait(vbuf, vsem, tv)
            @pl.when(j + NP < E)
            def _():
                start(v_hbm, vbuf, vsem, tv + NP)
            return v_comp(tv, j, H - 1, m, *c)
        l, acc = lax.fori_loop(0, E, last, (zl, za))
        out = finish(H - 1, l, acc, out)
        o_ref[0] = out[0:1].astype(bf16)

    def fn(A_x, A_k_cache, A_v_cache, A_wq, A_wo, B_x, B_w1, B_b1, B_w2):
        any_spec = pl.BlockSpec(memory_space=pl.ANY)
        return pl.pallas_call(
            kern,
            in_specs=[any_spec] * 8,
            out_specs=pl.BlockSpec(memory_space=pltpu.VMEM),
            out_shape=jax.ShapeDtypeStruct((1, 1, D), bf16),
            scratch_shapes=[
                pltpu.VMEM((RING, S, RW, DH), bf16), pltpu.VMEM((RING, S, RW, DH), bf16),
                pltpu.VMEM((2, E, 8, C), f32), pltpu.VMEM((H, 8, DH), f32),
                pltpu.VMEM((1, 1, D), bf16), pltpu.VMEM((D, H * DH), bf16), pltpu.VMEM((D, H * DH), bf16),
                pltpu.VMEM((D, F), bf16), pltpu.VMEM((F,), bf16), pltpu.VMEM((D, F), bf16),
                pltpu.SemaphoreType.DMA((NP,)), pltpu.SemaphoreType.DMA((NP,)), pltpu.SemaphoreType.DMA((6,)),
            ],
            compiler_params=pltpu.CompilerParams(vmem_limit_bytes=64 * 2**20, disable_bounds_checks=True),
            name=name, interpret=interpret,
        )(A_x, A_k_cache.reshape(H * S, L, DH), A_v_cache.reshape(H * S, L, DH), A_wq, A_wo.T, B_w1, B_b1, B_w2.T)
    return fn


_impl = build(NP=16, name="mha_mish_decode")


@jax.jit
def pallas_parallel_sum__mha_block_cached__dense_activation_mish__decode_kernel(
        A_x, A_k_cache, A_v_cache, A_wq, A_wo, B_x, B_w1, B_b1, B_w2):
    return _impl(A_x, A_k_cache, A_v_cache, A_wq, A_wo, B_x, B_w1, B_b1, B_w2)
```

```python
import jax
import jax.numpy as jnp
from jax import lax
from jax.experimental import pallas as pl
from jax.experimental.pallas import tpu as pltpu

H, SK, DH, D, F = 16, 16384, 256, 448, 1792
HD = H * DH
PAIRS = H // 2
F32, BF16 = jnp.float32, jnp.bfloat16
NT = (((1,), (1,)), ((), ()))

HI, LO = 0, 1

SEGS, HI_SEGS, ROWS = 8, 2, 32
KEYS = SEGS * ROWS
STEPS = SK // KEYS
HI_AHEAD, LO_AHEAD = 3, 16
RING = 32

W_SEGS = 4
W_ROWS = D // W_SEGS
W_HI_AHEAD = 2 * HI_AHEAD
ATTN_STEPS = 4 * (W_ROWS // 8)
MLP_STEPS = 2 * (W_ROWS // 8)
TAIL = HD - 2 * DH


def _kernel(x_hbm, k_hbm, v_hbm, wq_hbm, wo_hbm, wo_tail_hbm, w1_hbm, b1_hbm, w2_hbm, o_ref,
            ring, scores, proj, feat, bias, out, x_buf, b1_buf, w_in, w_out, w_tail, sems, misc_sems):

    def event_sem(step, e):
        return sems.at[(step & (RING - 1)) * 2 + e]

    def kv_start(src, pair, j, e, prio):
        g, n = (0, HI_SEGS) if prio == HI else (HI_SEGS, SEGS - HI_SEGS)
        row = pl.multiple_of((j & (STEPS - 1)) * ROWS, ROWS)
        pltpu.make_async_copy(
            src.at[pl.ds((pair * 2 + e) * SEGS + g, n), pl.ds(row, ROWS)],
            ring.at[j & (RING - 1), e, pl.ds(g, n)],
            event_sem(j, e),
        ).start(priority=prio)

    def kv_wait(j, e):
        buf = ring.at[j & (RING - 1), e]
        pltpu.make_async_copy(buf, buf, event_sem(j, e)).wait()

    def kv_block(j, e):
        return ring[j & (RING - 1), e].reshape(KEYS, DH)

    def w_refs(i, e, mlp, segs):
        if mlp:
            width = F // 2
            row, col, base = (i >> 1) * 8, (i & 1) * width, (HD, TAIL)[e]
            src = (w1_hbm, w2_hbm)[e]
        else:
            width = (HD // 4, TAIL // 4)[e]
            row, col, base = (i >> 2) * 8, (i & 3) * width, 0
            src = (wq_hbm, wo_hbm)[e]
        rows = pl.ds(pl.multiple_of(row, 8), 8)
        step = i - (MLP_STEPS if mlp else MLP_STEPS + ATTN_STEPS)
        return (src.at[segs, rows, pl.ds(pl.multiple_of(col, 128), width)],
                (w_in, w_out)[e].at[segs, rows, pl.ds(pl.multiple_of(col + base, 128), width)],
                event_sem(step, e))

    def w_start(i, e, prio, mlp):
        segs = pl.ds(0, 1) if prio == HI else pl.ds(1, W_SEGS - 1)
        pltpu.make_async_copy(*w_refs(i, e, mlp, segs)).start(priority=prio)

    def w_wait(i, e, mlp):
        _, buf, sem = w_refs(i, e, mlp, pl.ds(0, W_SEGS))
        pltpu.make_async_copy(buf, buf, sem).wait()

    def tail_rows(b):
        return pl.ds(128 * b, min(128, D - 128 * b))

    def tail_copy(b):
        return pltpu.make_async_copy(
            wo_tail_hbm.at[tail_rows(b), pl.ds(TAIL, 2 * DH)], w_tail.at[tail_rows(b)], misc_sems.at[b])

    def prime(i, _):
        for e in range(2):
            pl.when(i < W_HI_AHEAD)(lambda: w_start(i, e, HI, False))
            w_start(2 * i + e, 0, LO, False)
            w_start(2 * i + e, 1, LO, False)

    lax.fori_loop(0, LO_AHEAD // 2, prime, None)
    x_copy = pltpu.make_async_copy(x_hbm, x_buf, misc_sems.at[0])
    b1_copy = pltpu.make_async_copy(b1_hbm, b1_buf, misc_sems.at[1])
    x_copy.start()
    b1_copy.start()

    def attn_weights(i, _):
        for e in range(2):
            w_wait(i, e, False)
            for prio, n in ((HI, W_HI_AHEAD), (LO, LO_AHEAD)):
                pl.when(i + n < ATTN_STEPS)(lambda: w_start(i + n, e, prio, False))
                pl.when(i + n >= ATTN_STEPS)(lambda: w_start(i + n - ATTN_STEPS, e, prio, True))

    lax.fori_loop(0, ATTN_STEPS, attn_weights, None)

    x_copy.wait()
    b1_copy.wait()
    x = x_buf[0].astype(F32)
    centered = x - jnp.mean(x, axis=-1, keepdims=True)
    var = jnp.mean(centered * centered, axis=-1, keepdims=True)
    xn = jnp.broadcast_to(centered / jnp.sqrt(var + 1e-5), (8, D)).astype(BF16)
    out[...] = jnp.broadcast_to(x, (8, D))
    b1 = b1_buf[...].astype(F32).reshape(1, F)
    for c in range(F // DH):
        bias[c] = jnp.broadcast_to(b1[:, c * DH:(c + 1) * DH], (8, DH))

    def w_block(w, c):
        return w[:, :, pl.ds(pl.multiple_of(c * DH, DH), DH)].reshape(D, DH)

    def project(c):
        return jnp.dot(xn, w_block(w_in, c), preferred_element_type=F32)

    def mlp_weights(i, _):
        for e in range(2):
            w_wait(i, e, True)
            pl.when(i + W_HI_AHEAD < MLP_STEPS)(lambda: w_start(i + W_HI_AHEAD, e, HI, True))
            if e == 0:
                t = i + W_HI_AHEAD - MLP_STEPS
                pl.when(t >= 0)(lambda: kv_start(k_hbm, 0, t >> 1, t & 1, HI))
            pl.when(i + LO_AHEAD < MLP_STEPS)(lambda: w_start(i + LO_AHEAD, e, LO, True))
            pl.when(i + LO_AHEAD >= MLP_STEPS)(lambda: kv_start(k_hbm, 0, i + LO_AHEAD - MLP_STEPS, e, LO))

        @pl.when(jnp.logical_and((i & 7) == 4, i < 16))
        def _():
            proj[i >> 3] = project(i >> 3)

    lax.fori_loop(0, MLP_STEPS, mlp_weights, None)

    ahead = ((HI, HI_AHEAD), (LO, LO_AHEAD))

    def pair_body(p, _):
        q = [proj[e].astype(BF16) for e in range(2)]
        more = p + 1 < PAIRS

        def k_step(j, smax):
            smax = list(smax)
            for e in range(2):
                kv_wait(j, e)
                for prio, n in ahead:
                    pl.when(j + n < STEPS)(lambda: kv_start(k_hbm, p, j + n, e, prio))
                    pl.when(j + n >= STEPS)(lambda: kv_start(v_hbm, p, j + n, e, prio))
                s = lax.dot_general(q[e], kv_block(j, e), NT, preferred_element_type=F32)
                scores[j, e] = s
                smax[e] = jnp.maximum(smax[e], jnp.maximum(s[:, :128], s[:, 128:]))
            return tuple(smax)

        neg_inf = jnp.full((8, 128), -jnp.inf, F32)
        smax = lax.fori_loop(0, STEPS, k_step, (neg_inf, neg_inf))
        row_max = [jnp.max(m, axis=-1, keepdims=True) for m in smax]

        def v_step(j, carry):
            denom, acc = list(carry[0]), list(carry[1])
            for e in range(2):
                kv_wait(j, e)
                for prio, n in ahead:
                    pl.when(j + n < STEPS)(lambda: kv_start(v_hbm, p, j + n, e, prio))
                    pl.when(jnp.logical_and(j + n >= STEPS, more))(
                        lambda: kv_start(k_hbm, p + 1, j + n, e, prio))
                w = jnp.exp((scores[j, e] - row_max[e]) * (DH ** -0.5))
                denom[e] = denom[e] + (w[:, :128] + w[:, 128:])
                acc[e] = acc[e] + jnp.dot(w.astype(BF16), kv_block(j, e), preferred_element_type=F32)

            @pl.when((j & 7) == 7)
            def _():
                c = j >> 3

                @pl.when(jnp.logical_and(c < 3, p > 0))
                def _():
                    blk = jnp.where(c == 2, TAIL // DH + p - 1, 2 * (p - 1) + c)
                    out[...] += lax.dot_general(
                        feat[c].astype(BF16), w_block(w_out, blk), NT, preferred_element_type=F32)

                @pl.when(jnp.logical_and(jnp.logical_and(c >= 3, c < 6), more))
                def _():
                    proj[c - 3] = project(jnp.where(c == 5, H + p, 2 * (p + 1) + c - 3))

                @pl.when(jnp.logical_and(c == 6, more))
                def _():
                    h = proj[2] + bias[p]
                    softplus = jnp.log1p(jnp.exp(-jnp.abs(h))) + jnp.where(h > 0, h, 0.0)
                    feat[2] = h * jnp.tanh(softplus)

                @pl.when(jnp.logical_and(c == 6, jnp.logical_not(more)))
                def _():
                    for b in range(4):
                        tail_copy(b).start(priority=LO)

            return tuple(denom), tuple(acc)

        zero_denom, zero_acc = jnp.zeros((8, 128), F32), jnp.zeros((8, DH), F32)
        denom, acc = lax.fori_loop(0, STEPS, v_step, ((zero_denom,) * 2, (zero_acc,) * 2))
        for e in range(2):
            feat[e] = acc[e] / jnp.sum(denom[e], axis=-1, keepdims=True)

    lax.fori_loop(0, PAIRS, pair_body, None)

    last = jnp.concatenate([feat[0], feat[1]], axis=-1).astype(BF16)
    result = []
    for group in ((0, 1), (2, 3)):
        for b in group:
            tail_copy(b).wait()
        for b in group:
            r = tail_rows(b)
            full = out[:, r] + lax.dot_general(last, w_tail[r, :], NT, preferred_element_type=F32)
            result.append(full[0:1])
    o_ref[0] = jnp.concatenate(result, axis=-1).astype(o_ref.dtype)


@jax.jit
def pallas_parallel_sum__mha_block_cached__dense_activation_mish__decode_kernel(
    A_x: jax.Array,
    A_k_cache: jax.Array,
    A_v_cache: jax.Array,
    A_wq: jax.Array,
    A_wo: jax.Array,
    B_x: jax.Array,
    B_w1: jax.Array,
    B_b1: jax.Array,
    B_w2: jax.Array,
):
    del B_x
    return pl.pallas_call(
        _kernel,
        in_specs=[pl.BlockSpec(memory_space=pl.ANY)] * 9,
        out_specs=pl.BlockSpec(memory_space=pltpu.VMEM),
        out_shape=jax.ShapeDtypeStruct((1, 1, D), A_x.dtype),
        scratch_shapes=[
            pltpu.VMEM((RING, 2, SEGS, ROWS, DH), BF16),
            pltpu.VMEM((STEPS, 2, 8, KEYS), F32),
            pltpu.VMEM((3, 8, DH), F32),
            pltpu.VMEM((3, 8, DH), F32),
            pltpu.VMEM((F // DH, 8, DH), F32),
            pltpu.VMEM((8, D), F32),
            pltpu.VMEM((1, 1, D), BF16),
            pltpu.VMEM((F,), BF16),
            pltpu.VMEM((W_SEGS, W_ROWS, HD + F), BF16),
            pltpu.VMEM((W_SEGS, W_ROWS, TAIL + F), BF16),
            pltpu.VMEM((D, 2 * DH), BF16),
            pltpu.SemaphoreType.DMA((2 * RING,)),
            pltpu.SemaphoreType.DMA((4,)),
        ],
        compiler_params=pltpu.CompilerParams(
            vmem_limit_bytes=32 * 2**20,
            disable_semaphore_checks=True,
        ),
        name="mha_mish_decode",
    )(
        A_x,
        A_k_cache.reshape(H * SEGS, SK // SEGS, DH),
        A_v_cache.reshape(H * SEGS, SK // SEGS, DH),
        A_wq.reshape(W_SEGS, W_ROWS, HD),
        A_wo.T.reshape(W_SEGS, W_ROWS, HD),
        A_wo.T,
        B_w1.reshape(W_SEGS, W_ROWS, F),
        B_b1,
        B_w2.T.reshape(W_SEGS, W_ROWS, F),
    )
```
